```python
import os as _os
_os.environ.setdefault("JAX_PLATFORMS", "cpu")
import jax
import jax.numpy as jnp

def _softmax(x, axis=-1):
    return jax.nn.softmax(x, axis=axis)
def _gelu(x):
    return jax.nn.gelu(x, approximate=True)
def _silu(x):
    return jax.nn.silu(x)
def _sigmoid(x):
    return jax.nn.sigmoid(x)
def _layernorm(x, axis=-1, eps=1e-5):
    m = jnp.mean(x, axis=axis, keepdims=True)
    v = jnp.var(x, axis=axis, keepdims=True)
    return (x - m) / jnp.sqrt(v + eps)
def _scatter_add(tgt, idx, src, axis=0):
    return tgt.at[idx].add(src)
def _segment_sum(src, seg, n):
    return jax.ops.segment_sum(src, seg, n)
class _Rng:
    def __init__(self, key):
        self._k = key
    def _next(self):
        self._k, sub = jax.random.split(self._k)
        return sub
    def normal(self, shape):
        return jax.random.normal(self._next(), shape, dtype=jnp.bfloat16)
    def randint(self, lo, hi, shape):
        return jax.random.randint(self._next(), shape, lo, hi, dtype=jnp.int32)
    def uniform(self, shape, lo=0.0, hi=1.0):
        return jax.random.uniform(self._next(), shape, jnp.bfloat16, lo, hi)
    def permutation(self, n):
        return jax.random.permutation(self._next(), n)


kernel_name = 'standalone__linear_kernel_rfa__decode'

def setup_inputs():
    _rng = _Rng(jax.random.key(int.from_bytes(__import__("os").urandom(4), "little")))
    _w = (lambda a: (lambda t: t.astype(jnp.bfloat16) if jnp.issubdtype(t.dtype, jnp.floating) else t)(jnp.asarray(a)))
    B, H, Sq, Sk, D, M = 2, 16, 1, 16384, 256, 16
    return {
        "q": _w((lambda *s: _rng.normal(s) * 0.4)(B, H, Sq, D)),
        "k": _w((lambda *s: _rng.normal(s) * 1.6)(B, H, Sk, D)),
        "v": _w((lambda *s: _rng.normal(s) * 1.6)(B, H, Sk, D)),
        "omega": _w((lambda *s: _rng.normal(s) * 1.6)(M, D)),
    }

def reference(q, k, v, omega):
    d = q.shape[-1]
    m = omega.shape[0]
    scale = float(d) ** -0.25
    qs = q * scale
    ks = k * scale
    q_proj = jnp.einsum("bhsd,md->bhsm", qs, omega)
    k_proj = jnp.einsum("bhsd,md->bhsm", ks, omega)
    q_sq = 0.5 * jnp.einsum("bhsd,bhsd->bhs", qs, qs)[..., None]
    k_sq = 0.5 * jnp.einsum("bhsd,bhsd->bhs", ks, ks)[..., None]
    inv_sqrt_m = float(m) ** -0.5
    phi_q = jnp.exp(q_proj - q_sq) * inv_sqrt_m + 1e-6
    phi_k = jnp.exp(k_proj - k_sq) * inv_sqrt_m + 1e-6
    kv = jnp.einsum("bhsm,bhsd->bhmd", phi_k, v)
    z  = jnp.einsum("bhsm->bhm", phi_k)
    num = jnp.einsum("bhqm,bhmd->bhqd", phi_q, kv)
    den = jnp.einsum("bhqm,bhm->bhq", phi_q, z)[..., None] + 1e-6
    return num / den
```

```python
import jax
import jax.numpy as jnp
from jax import lax
import jax.experimental.pallas as pl
import jax.experimental.pallas.tpu as pltpu

ROWS = 512
NBUF = 8
SPLIT = 8

_NT = (((1,), (1,)), ((), ()))


def _kernel(q_ref, om_ref, k_hbm, v_hbm, o_ref, kb, vb, ob, sems):
    BH, D = q_ref.shape
    M = om_ref.shape[0]
    S = k_hbm.shape[1]
    cph = S // ROWS
    n = BH * cph
    scale = float(D) ** -0.25
    half_s2 = 0.5 * scale * scale
    c = float(M) ** -0.5
    r = ROWS // SPLIT
    hs = SPLIT // 2

    def start(i, slot):
        h = i // cph
        s0 = (i % cph) * ROWS

        def one(src, dst, t, p):
            pltpu.make_async_copy(
                src.at[h, pl.ds(pl.multiple_of(s0 + t * r, r), r)],
                dst.at[slot, pl.ds(t * r, r)],
                sems.at[slot],
            ).start(priority=p)

        for t in range(hs):
            one(k_hbm, kb, t, 0)
            one(k_hbm, kb, t + hs, 1)
            one(v_hbm, vb, t, 0)
            one(v_hbm, vb, t + hs, 1)

    def wait(slot):
        pltpu.make_async_copy(kb.at[slot], kb.at[slot], sems.at[slot]).wait()
        pltpu.make_async_copy(vb.at[slot], vb.at[slot], sems.at[slot]).wait()

    for i in range(NBUF - 1):
        start(i, i)

    om = om_ref[...]
    ones = jnp.ones((M, 128), jnp.bfloat16)

    q = q_ref[...]
    qf = q.astype(jnp.float32)
    qp = lax.dot_general(om, q, _NT, preferred_element_type=jnp.float32)
    q2 = qf * qf
    hi = q2.astype(jnp.bfloat16)
    lo = (q2 - hi.astype(jnp.float32)).astype(jnp.bfloat16)
    o2 = jnp.ones((M, D), jnp.bfloat16)
    qs = (lax.dot_general(o2, hi, _NT, preferred_element_type=jnp.float32)
          + lax.dot_general(o2, lo, _NT, preferred_element_type=jnp.float32))
    pqT = jnp.exp(qp * scale - half_s2 * qs) * c + 1e-6
    lane = lax.broadcasted_iota(jnp.int32, (M, BH), 1)

    def phi(slot):
        k = kb[slot]
        p = lax.dot_general(om, k, _NT, preferred_element_type=jnp.float32)
        kf = k.astype(jnp.float32)
        k2 = kf * kf
        a = k2[:, 0:128]
        for t in range(1, D // 128):
            a = a + k2[:, t * 128:(t + 1) * 128]
        ss = lax.dot_general(ones, a.astype(jnp.bfloat16), _NT,
                             preferred_element_type=jnp.float32)
        return (jnp.exp(p * scale - half_s2 * ss) * c + 1e-6).astype(jnp.bfloat16)

    def head(h, pb):
        def body(j, carry):
            pb, kv, z = carry
            i = h * cph + j
            nx = i + NBUF - 1

            @pl.when(nx < n)
            def _():
                start(nx, nx % NBUF)

            @pl.when(i + 1 < n)
            def _():
                wait((i + 1) % NBUF)

            pn = phi((i + 1) % NBUF)
            kv = kv + jnp.dot(pb, vb[i % NBUF], preferred_element_type=jnp.float32)
            pf = pb.astype(jnp.float32)
            for t in range(ROWS // 128):
                z = z + pf[:, t * 128:(t + 1) * 128]
            return pn, kv, z

        pb, kv, z = lax.fori_loop(
            0, cph, body,
            (pb, jnp.zeros((M, D), jnp.float32), jnp.zeros((M, 128), jnp.float32)))
        pq = jnp.sum(jnp.where(lane == h, pqT, 0.0), axis=1, keepdims=True)
        num = jnp.sum(pq * kv, axis=0, keepdims=True)
        den = jnp.sum(pq * jnp.sum(z, axis=1, keepdims=True), axis=0, keepdims=True) + 1e-6
        ob[pl.ds(h, 1), :] = num / den
        return pb

    wait(0)
    lax.fori_loop(0, BH, head, phi(0))
    o_ref[...] = ob[...].astype(o_ref.dtype)


@jax.jit
def pallas_standalone__linear_kernel_rfa__decode_kernel(
    q: jax.Array,
    k: jax.Array,
    v: jax.Array,
    omega: jax.Array,
):
    B, H, Sq, D = q.shape
    S = k.shape[2]
    assert Sq == 1 and S % ROWS == 0 and D % 128 == 0
    assert B * H * (S // ROWS) >= NBUF
    out = pl.pallas_call(
        _kernel,
        in_specs=[pl.BlockSpec(memory_space=pltpu.VMEM)] * 2
        + [pl.BlockSpec(memory_space=pl.ANY)] * 2,
        out_specs=pl.BlockSpec(memory_space=pltpu.VMEM),
        out_shape=jax.ShapeDtypeStruct((B * H, D), q.dtype),
        scratch_shapes=[
            pltpu.VMEM((NBUF, ROWS, D), k.dtype),
            pltpu.VMEM((NBUF, ROWS, D), v.dtype),
            pltpu.VMEM((B * H, D), jnp.float32),
            pltpu.SemaphoreType.DMA((NBUF,)),
        ],
        compiler_params=pltpu.CompilerParams(vmem_limit_bytes=64 * 1024 * 1024),
    )(q.reshape(B * H, D), omega, k.reshape(B * H, S, D), v.reshape(B * H, S, D))
    return out.reshape(B, H, Sq, D)
```
